```python
import os as _os
_os.environ.setdefault("JAX_PLATFORMS", "cpu")
import jax
import jax.numpy as jnp

def _softmax(x, axis=-1):
    return jax.nn.softmax(x, axis=axis)
def _gelu(x):
    return jax.nn.gelu(x, approximate=True)
def _silu(x):
    return jax.nn.silu(x)
def _sigmoid(x):
    return jax.nn.sigmoid(x)
def _layernorm(x, axis=-1, eps=1e-5):
    m = jnp.mean(x, axis=axis, keepdims=True)
    v = jnp.var(x, axis=axis, keepdims=True)
    return (x - m) / jnp.sqrt(v + eps)
def _scatter_add(tgt, idx, src, axis=0):
    return tgt.at[idx].add(src)
def _segment_sum(src, seg, n):
    return jax.ops.segment_sum(src, seg, n)
class _Rng:
    def __init__(self, key):
        self._k = key
    def _next(self):
        self._k, sub = jax.random.split(self._k)
        return sub
    def normal(self, shape):
        return jax.random.normal(self._next(), shape, dtype=jnp.bfloat16)
    def randint(self, lo, hi, shape):
        return jax.random.randint(self._next(), shape, lo, hi, dtype=jnp.int32)
    def uniform(self, shape, lo=0.0, hi=1.0):
        return jax.random.uniform(self._next(), shape, jnp.bfloat16, lo, hi)
    def permutation(self, n):
        return jax.random.permutation(self._next(), n)


kernel_name = 'parallel_sum__spectral_gfnet__glu_gated_swiglu__prompt'

def setup_inputs():
    _rng = _Rng(jax.random.key(int.from_bytes(__import__("os").urandom(4), "little")))
    _w = (lambda a: (lambda t: t.astype(jnp.bfloat16) if jnp.issubdtype(t.dtype, jnp.floating) else t)(jnp.asarray(a)))
    def _A_setup():
        B, S, D = 1, 2048, 512
        Df = D // 2 + 1
        return {
            "x": _w((lambda *s: _rng.normal(s) * 0.05)(B, S, D)),
            "w_r": _w((lambda *s: _rng.normal(s) * 0.2)(S, Df) * 0.02),
            "w_i": _w((lambda *s: _rng.normal(s) * 0.2)(S, Df) * 0.02),
        }
    _A_in = _A_setup()

    def _B_setup():
        B, S, D, F = 1, 2048, 512, 1376
        return {
            "x": _w((lambda *s: _rng.normal(s) * 0.05)(B, S, D)),
            "w1": _w((lambda *s: _rng.normal(s) * 0.05)(D, F) * (2.0 / D) ** 0.5),
            "w3": _w((lambda *s: _rng.normal(s) * 0.05)(D, F) * (2.0 / D) ** 0.5),
            "w2": _w((lambda *s: _rng.normal(s) * 0.05)(F, D) * (2.0 / F) ** 0.5),
        }
    _B_in = _B_setup()

    return {
        "A_x": _A_in["x"],
        "A_w_r": _A_in["w_r"],
        "A_w_i": _A_in["w_i"],
        "B_x": _B_in["x"],
        "B_w1": _B_in["w1"],
        "B_w3": _B_in["w3"],
        "B_w2": _B_in["w2"],
    }

def reference(A_x, A_w_r, A_w_i, B_x, B_w1, B_w3, B_w2):
    def _A_ref(x, w_r, w_i):
        B, S, D = x.shape
        X = (lambda x, axes=(-2,-1): jnp.fft.rfft2(x.astype(jnp.float32), axes=axes))(x, axes=(-2, -1))
        W = w_r + 1j * w_i
        X = X * W
        y = (lambda x, s, axes=(-2,-1): jnp.fft.irfft2(x, s=s, axes=axes).astype(jnp.bfloat16))(X, (S, D), axes=(-2, -1))
        return y

    def _B_ref(x, w1, w3, w2):
        gate = jnp.einsum("bsd,df->bsf", x, w1)
        up = jnp.einsum("bsd,df->bsf", x, w3)
        h = _silu(gate) * up
        out = jnp.einsum("bsf,fd->bsd", h, w2)
        return out

    x = A_x
    xn = _layernorm(x, axis=-1)
    return x + _A_ref(xn, A_w_r, A_w_i) + _B_ref(xn, B_w1, B_w3, B_w2)
```

```python
import numpy as np
import jax
import jax.numpy as jnp
import jax.experimental.pallas as pl
import jax.experimental.pallas.tpu as pltpu

S, D, F = 2048, 512, 1376
BF, F32 = jnp.bfloat16, jnp.float32
M1 = 512


def _consts():
    n = np.arange(256)[:, None]
    j = np.arange(128)
    fd, fi = [], []
    for d in (2 * j, 2 * j + 1):
        th = 2 * np.pi * n * d[None, :] / D
        f = np.concatenate([np.cos(th), -np.sin(th)], 1)
        g = f.T * (2.0 / D)
        if d[0] == 0:
            f[:, 128] = (-1.0) ** n[:, 0]
            g[0] = 1.0 / D
            g[128] = (-1.0) ** n[:, 0] / D
        fd.append(f)
        fi.append(g)
    blk = lambda c: np.block([[c.real, -c.imag], [c.imag, c.real]])
    gf, gi = [], []
    q = np.arange(64)
    for k1 in range(32):
        c = np.exp(-2j * np.pi * (k1 + 32 * q[:, None]) * q[None, :] / S)
        gf.append(blk(c) / 32)
        gi.append(blk(c.conj().T) / 64)
    a = np.arange(16)
    f16 = np.exp(-2j * np.pi * a[:, None] * a[None, :] / 16)
    tw = np.exp(-2j * np.pi * a[:, None] * j[None, :] / S)
    f128 = np.exp(-2j * np.pi * j[:, None] * j[None, :] / 128)
    rb = lambda c: np.block([[c.real, c.imag], [-c.imag, c.real]])
    s16 = np.zeros((2, 32, 128))
    s16[0, :16, :16], s16[0, 16:, :16] = f16.real, f16.imag
    s16[1, :16, :16], s16[1, :16, 16:32] = f16.real / S, f16.imag / S
    b = lambda x: np.asarray(x, np.float32).astype(BF)
    return (b(fd + fi + [rb(f128), rb(f128.conj())]), b(gf + gi), b(s16),
            np.stack([tw.real, tw.imag]).astype(np.float32))


def _tw(z, m, n, sg):
    r, i = z
    m %= n
    if m == 0:
        return z
    if 4 * m == n:
        return (-i, r) if sg > 0 else (i, -r)
    c, s = float(np.cos(2 * np.pi * m / n)), float(sg * np.sin(2 * np.pi * m / n))
    return (r * c - i * s, r * s + i * c)


def _fft(z, sg):
    n = len(z)
    if n == 1:
        return z
    e, o = _fft(z[0::2], sg), _fft(z[1::2], sg)
    out = [None] * n
    for k in range(n // 2):
        a = e[k]
        if 4 * k == n:
            p, m = (a[0] - o[k][1], a[1] + o[k][0]), (a[0] + o[k][1], a[1] - o[k][0])
            if sg < 0:
                p, m = m, p
        else:
            t = _tw(o[k], k, n, sg)
            p, m = (a[0] + t[0], a[1] + t[1]), (a[0] - t[0], a[1] - t[1])
        out[k], out[k + n // 2] = p, m
    return out


def _dot(a, b):
    return jnp.dot(a, b, preferred_element_type=F32)


def _dnt(a, b):
    return jax.lax.dot_general(a, b, (((1,), (1,)), ((), ())), preferred_element_type=F32)


def _kernel(x_h, wr_h, wi_h, w1_h, w3_h, w2_h, fd_h, g_h, s16, tw, o_h,
            x, w, wn, wn2, w1, w3, w2, fd, g, h, acc, u, v, ny, o, sem):
    cp = []
    nb = S // M1
    for i in range(nb):
        cp.append((x_h.at[0, pl.ds(i * M1, M1)], x.at[pl.ds(i * M1, M1)]))
    cp[1:1] = [(fd_h, fd)]
    cp += [(w1_h, w1), (w3_h, w3)]
    cp.append((w2_h, w2))
    cp.append((g_h, g))
    cp += [(wr_h, wn.at[0]), (wi_h, wn.at[1])]
    cp = [pltpu.make_async_copy(a, b, sem.at[i]) for i, (a, b) in enumerate(cp)]
    for c in cp[:nb + 3]:
        c.start()
    cp[1].wait()
    lane = jax.lax.broadcasted_iota(jnp.int32, (128, 128), 1)

    def p1(i, _):
        r0 = pl.multiple_of(i * M1, M1)
        rows = pl.ds(r0, M1)
        pltpu.make_async_copy(x.at[rows], x.at[rows], sem.at[jnp.where(i == 0, 0, i + 1)]).wait()
        xv = x[rows, :].astype(F32)
        xc = xv - jnp.mean(xv, -1, keepdims=True)
        xn = xc * jax.lax.rsqrt(jnp.mean(xc * xc, -1, keepdims=True) + 1e-5)
        lo, hi = xn[:, :256], xn[:, 256:]
        e = _dot((lo + hi).astype(BF), fd[0])
        od = _dot((lo - hi).astype(BF), fd[1])
        u[0, rows, :] = e[:, :128]
        u[2, rows, :] = od[:, :128]
        u[3, rows, :] = od[:, 128:]
        for b in range(M1 // 128):
            t = e[128 * b:128 * b + 128, 128:]
            u[1, pl.ds(r0 + 128 * b, 128), :] = jnp.where(lane == 0, 0.0, t)
            ny[i * (M1 // 128) + b] = t.T[:8]
        o[rows, :] = xn.astype(BF)
        return 0

    jax.lax.fori_loop(0, nb, p1, 0)
    cp[nb + 1].wait()
    cp[nb + 2].wait()
    for c in cp[nb + 3:]:
        c.start()

    def p1(i, _):
        rows = pl.ds(pl.multiple_of(i * M1, M1), M1)
        xb = o[rows, :]
        for c0 in range(0, F, 256):
            cs = slice(c0, min(c0 + 256, F))
            ga, up = _dnt(xb, w1[cs, :]), _dnt(xb, w3[cs, :])
            h[rows, cs] = (ga * up / (1.0 + jnp.exp(-ga))).astype(BF)
        return 0

    jax.lax.fori_loop(0, nb, p1, 0)
    for c in cp[nb + 3:]:
        c.wait()

    def down(i, c):
        cs = slice(128 * c, 128 * c + 256)
        rows = pl.ds(pl.multiple_of(i * 256, 256), 256)
        def gen():
            a = x[rows, cs].astype(F32)
            for k0 in range(0, F, 256):
                ks = slice(k0, min(k0 + 256, F))
                a = a + _dot(h[rows, ks], w2[ks, cs])
                if k0 + 256 >= F:
                    acc[rows, cs] = a
                yield
        todo[:] = [gen()]

    todo = []

    def step():
        next(todo[0], None)

    def fft32(r, t, sg, load, store):
        for hf in range(2):
            step()
            rr = pl.ds(pl.multiple_of(r + 8 * hf, 8), 8)
            for b in range(8):
                z = _fft([load(8 * a + b, t, rr) for a in range(4)], sg)
                for c in range(4):
                    y = _tw(z[c], b * c, 32, sg)
                    v[c, b, 0, 8 * hf:8 * hf + 8], v[c, b, 1, 8 * hf:8 * hf + 8] = y
        step()
        for c in range(4):
            z = _fft([(v[c, b, 0], v[c, b, 1]) for b in range(8)], sg)
            for e in range(8):
                store(c + 4 * e, t, z[e])

    def p2(i, _):
        r = pl.multiple_of(i * 16, 16)

        def st(k, t, z):
            for c in range(2):
                o[pl.ds(64 * k + r, 16), pl.ds(256 * c + 128 * t, 128)] = z[c].astype(BF)
        for t in range(2):
            fft32(r, t, -1, lambda n, t, rr: tuple(
                u[2 * t + c, pl.ds(64 * n + rr.start, 8), :] for c in range(2)), st)
        for b in range(4):
            k0 = pl.multiple_of(i * 512 + b * 128, 128)
            for c in range(2):
                w[c, pl.ds(k0, 128), :] = pltpu.bitcast(wn[c, :256, pl.ds(k0, 128)], jnp.int32).T
                q = wn[c, 256:257, pl.ds(k0, 128)].astype(F32)
                wn2[c, pl.ds(k0, 128), :] = jnp.broadcast_to(q, (128, 128)).T
        return 0

    jax.lax.fori_loop(0, 2, lambda i, _: (down(0 + i, 0), p2(2 * i, 0), down(0 + i, 2), p2(2 * i + 1, 0))[1], 0)

    def p3(i, _):
        for jj in range(2):
            j = 2 * i + jj
            for hf in range(2):
                k = 2 * j + hf
                step()
                wt = [w[c, pl.ds(k, 64, stride=32), :] for c in range(2)]
                wr, wi = [pltpu.bitcast(jnp.concatenate([t << 16, t & -65536], 1), F32) for t in wt]
                rows = pl.ds(pl.multiple_of(k * 64, 64), 64)
                z = _dot(g[k], jnp.concatenate([o[rows, :256], o[rows, 256:]], 0))
                step()
                zr, zi = z[:64], z[64:]
                y = jnp.concatenate([zr * wr - zi * wi, zr * wi + zi * wr], 0).astype(BF)
                y = _dot(g[32 + k], y)
                for t in range(2):
                    for c in range(2):
                        u[2 * t + c, rows, :] = y[64 * c:64 * c + 64, 128 * t:128 * t + 128]
        return 0

    jax.lax.fori_loop(0, 4, lambda i, _: (down(2 + i, 0), p3(2 * i, 0), down(2 + i, 2), p3(2 * i + 1, 0))[1], 0)

    wq = []
    for c in range(2):
        wq.append(jnp.concatenate(
            [wn2[c, pl.ds(j, 128, stride=16), :].T[:1] for j in range(16)], 0))
    r = jnp.concatenate([ny[b, :1] for b in range(16)] + [jnp.zeros((112, 128), F32)], 0)
    t = _dot(s16[0], r.astype(BF))
    cm = lambda a, b, c, d: jnp.concatenate([a * c - b * d, a * d + b * c], 1)
    t = _dot(cm(t[:16], t[16:], tw[0], tw[1]).astype(BF), fd[4])
    t = _dot(cm(t[:, :128], t[:, 128:], wq[0], wq[1]).astype(BF), fd[5])
    t = cm(t[:, :128], t[:, 128:], tw[0], -tw[1])
    t = jnp.concatenate([t[:, :128], t[:, 128:], jnp.zeros((96, 128), F32)], 0)
    t = _dot(s16[1], t.astype(BF))
    for b in range(16):
        ny[b] = jnp.broadcast_to(t[b:b + 1], (8, 128))

    def p4(i, _):
        r = pl.multiple_of(i * 16, 16)

        def st(k, t, z):
            for c in range(2):
                o[pl.ds(64 * k + r, 16), pl.ds(256 * t + 128 * c, 128)] = z[c].astype(BF)
        for t in range(2):
            fft32(r, t, 1, lambda n, t, rr: tuple(
                u[2 * t + c, pl.ds(64 * n + rr.start, 8), :] for c in range(2)), st)
        return 0

    jax.lax.fori_loop(0, 2, lambda i, _: (down(6 + i, 0), p4(2 * i, 0), down(6 + i, 2), p4(2 * i + 1, 0))[1], 0)

    def p5(i, _):
        r0 = pl.multiple_of(i * 256, 256)
        rows = pl.ds(r0, 256)
        nq = jnp.concatenate([jnp.broadcast_to(ny[2 * i + b, :1], (128, 128)).T for b in range(2)], 0)
        l2 = jax.lax.broadcasted_iota(jnp.int32, (256, 128), 1)
        im = jnp.where(l2 == 0, nq, o[rows, 128:256].astype(F32)).astype(BF)
        a = _dot(jnp.concatenate([o[rows, :128], im], 1), fd[2])
        b = _dot(o[rows, 256:], fd[3])
        x[rows, :256] = (acc[rows, :256] + (a + b)).astype(BF)
        x[rows, 256:] = (acc[rows, 256:] + (a - b)).astype(BF)
        pltpu.make_async_copy(x.at[rows], o_h.at[0, rows], sem.at[0]).start()
        return 0

    jax.lax.fori_loop(0, 8, p5, 0, unroll=4)
    pltpu.make_async_copy(x, o_h.at[0], sem.at[0]).wait()


@jax.jit
def pallas_parallel_sum__spectral_gfnet__glu_gated_swiglu__prompt_kernel(
        A_x, A_w_r, A_w_i, B_x, B_w1, B_w3, B_w2):
    del B_x
    V = pltpu.VMEM
    hbm = pl.BlockSpec(memory_space=pltpu.HBM)
    vm = pl.BlockSpec(memory_space=pltpu.VMEM)
    return pl.pallas_call(
        _kernel,
        out_shape=jax.ShapeDtypeStruct((1, S, D), BF),
        in_specs=[hbm] * 8 + [vm] * 2,
        out_specs=hbm,
        scratch_shapes=[
            V((S, D), BF), V((2, S, 128), jnp.int32), V((2, 257, S), BF), V((2, S, 128), F32),
            V((F, D), BF), V((F, D), BF), V((F, D), BF), V((6, 256, 256), BF),
            V((64, 128, 128), BF), V((S, F), BF), V((S, D), F32), V((4, S, 128), F32),
            V((4, 8, 2, 16, 128), F32), V((16, 8, 128), F32), V((S, D), BF),
            pltpu.SemaphoreType.DMA((32,)),
        ],
        compiler_params=pltpu.CompilerParams(vmem_limit_bytes=100 << 20),
    )(A_x, A_w_r.T, A_w_i.T, B_w1.T, B_w3.T, B_w2, *_consts())
```
